```python
import os as _os
_os.environ.setdefault("JAX_PLATFORMS", "cpu")
import jax
import jax.numpy as jnp

def _softmax(x, axis=-1):
    return jax.nn.softmax(x, axis=axis)
def _gelu(x):
    return jax.nn.gelu(x, approximate=True)
def _silu(x):
    return jax.nn.silu(x)
def _sigmoid(x):
    return jax.nn.sigmoid(x)
def _layernorm(x, axis=-1, eps=1e-5):
    m = jnp.mean(x, axis=axis, keepdims=True)
    v = jnp.var(x, axis=axis, keepdims=True)
    return (x - m) / jnp.sqrt(v + eps)
def _scatter_add(tgt, idx, src, axis=0):
    return tgt.at[idx].add(src)
def _segment_sum(src, seg, n):
    return jax.ops.segment_sum(src, seg, n)
class _Rng:
    def __init__(self, key):
        self._k = key
    def _next(self):
        self._k, sub = jax.random.split(self._k)
        return sub
    def normal(self, shape):
        return jax.random.normal(self._next(), shape, dtype=jnp.bfloat16)
    def randint(self, lo, hi, shape):
        return jax.random.randint(self._next(), shape, lo, hi, dtype=jnp.int32)
    def uniform(self, shape, lo=0.0, hi=1.0):
        return jax.random.uniform(self._next(), shape, jnp.bfloat16, lo, hi)
    def permutation(self, n):
        return jax.random.permutation(self._next(), n)


kernel_name = 'standalone__detection_seg_fpn_lateral__vision'

def setup_inputs():
    _rng = _Rng(jax.random.key(int.from_bytes(__import__("os").urandom(4), "little")))
    _w = (lambda a: (lambda t: t.astype(jnp.bfloat16) if jnp.issubdtype(t.dtype, jnp.floating) else t)(jnp.asarray(a)))
    H = W = (256 // 2) * 2
    C = 384
    k = 1
    return {
        "c_fine": _w((lambda *s: _rng.normal(s) * 0.05)(1, H, W, C)),
        "p_coarse": _w((lambda *s: _rng.normal(s) * 0.05)(1, H // 2, W // 2, C)),
        "w_lat": _w((lambda *s: _rng.normal(s) * 0.05)(C, C)),
        "w_out": _w((lambda *s: _rng.normal(s) * 0.05)(k, k, C, C)),
    }

def reference(c_fine, p_coarse, w_lat, w_out):
    B, H, W, C = c_fine.shape
    k = 1
    lat = jnp.einsum("bhwc,cd->bhwd", c_fine, w_lat)
    up = jnp.repeat(jnp.repeat(p_coarse, 2, axis=1), 2, axis=2)
    m = lat + up
    pad = k // 2
    mp = jnp.pad(m, ((0, 0), (pad, pad), (pad, pad), (0, 0)))
    o = None
    for di in range(k):
        for dj in range(k):
            t = jnp.einsum("bhwc,cd->bhwd", mp[:, di:di + H, dj:dj + W, :], w_out[di, dj])
            o = t if o is None else o + t
    return o
```

```python
import jax
import jax.numpy as jnp
from jax import lax
from jax.experimental import pallas as pl
from jax.experimental.pallas import tpu as pltpu

def build(TP=4, S=8, D=1024, R=32, I0=19, KW=16, BURST=24, RP=1, WP=0, NOCOMP=False, NOBC=False, NOSC=False,
          TWOLOOP=True, TAILROWS=512, CLASSES=((0, 1), (2, 2), (8, 4))):
    def f(c_fine, p_coarse, w_lat, w_out):
        B, H, W, C = c_fine.shape
        M = B * H * W
        W2 = W // 2
        PR = 2 * W
        J = D // PR
        G = M // (S * D)
        SB = S // TP
        NU = G * J * SB
        PERS = PR // R
        NW = G * J * PERS
        NT = C // 128
        assert SB * TP == S and J * PR == D

        chunks = []
        u = 0
        while u <= I0:
            size = [sz for (st, sz) in CLASSES if u >= st][-1]
            chunks.append((u, size)); u += size
        rest0 = u
        assert rest0 % SB == 0
        NCH = len(chunks)

        def kern(c_hbm, p_hbm, wl_hbm, wo_hbm, o_hbm, cbuf, pbuf, obuf, wl, wo, wf, qs, csem, wsem, rsem, tsem, osem):
            def unit_slices(u, size):
                sl = u // SB
                g = sl // J; j = sl % J
                if size < SB:
                    assert size == 1
                    sb = u % SB
                    return (g, pl.ds(sb * TP, TP), pl.ds(j, 1))
                m = size // SB
                return (g, slice(None), pl.ds(j, m))
            def rd(u, size, sem):
                idx = unit_slices(u, size)
                return [pltpu.make_async_copy(p_hbm.at[idx], pbuf.at[idx], sem),
                        pltpu.make_async_copy(c_hbm.at[idx], cbuf.at[idx], sem)]
            def o_cp(jj):
                sl = jj // PERS
                g = sl // J
                off = pl.multiple_of((jj % (J * PERS)) * R, R)
                return pltpu.make_async_copy(obuf.at[g, :, pl.ds(off, R)], o_hbm.at[g, :, pl.ds(off, R)], osem)
            rest = []
            sl = rest0 // SB
            while sl < G * J:
                g = sl // J; j = sl % J
                m = J - j
                idx = (g, slice(None), pl.ds(j, m))
                last = (sl + m == G * J)
                rest.append(pltpu.make_async_copy(p_hbm.at[idx], pbuf.at[idx], rsem))
                if not last:
                    rest.append(pltpu.make_async_copy(c_hbm.at[idx], cbuf.at[idx], rsem))
                else:
                    i1 = (g, pl.ds(0, S - 1), pl.ds(j, m))
                    rest.append(pltpu.make_async_copy(c_hbm.at[i1], cbuf.at[i1], rsem))
                    if m > 1:
                        i2 = (g, S - 1, pl.ds(j, m - 1))
                        rest.append(pltpu.make_async_copy(c_hbm.at[i2], cbuf.at[i2], rsem))
                    if TAILROWS < PR:
                        i3 = (g, S - 1, J - 1, pl.ds(0, PR - TAILROWS))
                        rest.append(pltpu.make_async_copy(c_hbm.at[i3], cbuf.at[i3], rsem))
                    i4 = (g, S - 1, J - 1, pl.ds(PR - TAILROWS, TAILROWS))
                    tail = pltpu.make_async_copy(c_hbm.at[i4], cbuf.at[i4], tsem)
                sl += m

            wl_cp = pltpu.make_async_copy(wl_hbm, wl, wsem.at[0])
            wo_cp = pltpu.make_async_copy(wo_hbm, wo, wsem.at[1])
            wl_cp.start(0); wo_cp.start(0)
            for k, (st, sz) in enumerate(chunks):
                for d in rd(st, sz, csem.at[k]):
                    d.start(RP)
            for d in rest:
                d.start(RP)
            tail.start(RP)
            wl_cp.wait(); wo_cp.wait()
            wf[...] = jnp.dot(wl[...], wo[...], preferred_element_type=jnp.float32).astype(jnp.bfloat16)

            def compute(u):
                if NOCOMP:
                    return
                sl = u // SB
                g = sl // J; j = sl % J
                s0 = (u % SB) * TP
                p = pbuf[g, pl.ds(s0, TP), j].reshape(TP * W2, C)
                q = jnp.dot(p, wo[...], preferred_element_type=jnp.float32)
                for n in range(NT):
                    qn = q[:, n*128:(n+1)*128]
                    qs[n, pl.ds(0, TP * W2, stride=2), :] = qn
                    qs[n, pl.ds(1, TP * W2, stride=2), :] = qn
                for t in range(TP):
                    qu = jnp.concatenate([qs[n, pl.ds(t * W, W), :] for n in range(NT)], axis=1)
                    for r in range(2):
                        c = cbuf[g, s0 + t, j, pl.ds(r * W, W), :]
                        res = (jnp.dot(c, wf[...], preferred_element_type=jnp.float32) + qu).astype(jnp.bfloat16)
                        obuf[g, s0 + t, pl.ds(pl.multiple_of(j * PR + r * W, W), W), :] = res

            def chunk_waits(u):
                kbase = 0
                bounds = [st for (st, sz) in CLASSES] + [rest0]
                for ci, (st, sz) in enumerate(CLASSES):
                    en = min(bounds[ci + 1], rest0)
                    if st >= rest0: break
                    cond = (u >= st) & (u < en)
                    if sz > 1:
                        cond = cond & ((u - st) % sz == 0)
                    k = kbase + (u - st) // sz
                    @pl.when(cond)
                    def _(k=k, st=st, sz=sz):
                        for d in rd(st, sz, csem.at[k]):
                            d.wait()
                    kbase += (en - st + sz - 1) // sz

            def switch():
                for d in rest:
                    d.wait()
                for jj in range(BURST):
                    o_cp(jj).start(WP)

            def issue(u):
                base = BURST + (u - I0 - 1) * KW
                for k in range(KW):
                    o_cp(base + k).start(WP)

            if TWOLOOP:
                def bodyA(u, _):
                    chunk_waits(u)
                    compute(u)
                    return 0
                lax.fori_loop(0, I0 + 1, bodyA, 0)
                switch()
                tail.wait()
                def bodyB(u, _):
                    issue(u)
                    compute(u)
                    return 0
                lax.fori_loop(I0 + 1, NU, bodyB, 0)
            else:
                def body(u, _):
                    chunk_waits(u)
                    @pl.when(u > I0)
                    def _():
                        issue(u)
                    @pl.when(u == NU - 1)
                    def _():
                        tail.wait()
                    compute(u)
                    @pl.when(u == I0)
                    def _():
                        switch()
                    return 0
                lax.fori_loop(0, NU, body, 0)
            done = BURST + (NU - I0 - 1) * KW
            assert done <= ((NU - 1) // SB) * PERS, (done, NW)
            for jj in range(done, NW):
                o_cp(jj).start(WP)
            pltpu.make_async_copy(obuf, o_hbm, osem).wait()

        c5 = c_fine.reshape(G, S, J, PR, C); p5 = p_coarse.reshape(G, S, J, W2, C); wo2 = w_out.reshape(C, C)
        out = pl.pallas_call(
            kern,
            in_specs=[pl.BlockSpec(memory_space=pl.ANY)] * 4,
            out_specs=pl.BlockSpec(memory_space=pl.ANY),
            out_shape=jax.ShapeDtypeStruct((G, S, D, C), c_fine.dtype),
            scratch_shapes=[
                pltpu.VMEM((G, S, J, PR, C), jnp.bfloat16), pltpu.VMEM((G, S, J, W2, C), jnp.bfloat16), pltpu.VMEM((G, S, D, C), jnp.bfloat16),
                pltpu.VMEM((C, C), jnp.bfloat16), pltpu.VMEM((C, C), jnp.bfloat16), pltpu.VMEM((C, C), jnp.bfloat16),
                pltpu.VMEM((NT, TP * W, 128), jnp.float32),
                pltpu.SemaphoreType.DMA((NCH,)), pltpu.SemaphoreType.DMA((2,)), pltpu.SemaphoreType.DMA, pltpu.SemaphoreType.DMA, pltpu.SemaphoreType.DMA,
            ],
            compiler_params=pltpu.CompilerParams(vmem_limit_bytes=124 * 1024 * 1024, disable_bounds_checks=NOBC, disable_semaphore_checks=NOSC),
        )(c5, p5, w_lat, wo2)
        return out.reshape(B, H, W, C)
    return jax.jit(f)


_impl = build()


@jax.jit
def pallas_standalone__detection_seg_fpn_lateral__vision_kernel(c_fine, p_coarse, w_lat, w_out):
    return _impl(c_fine, p_coarse, w_lat, w_out)
```

```python
import jax
import jax.numpy as jnp
from jax import lax
import jax.experimental.pallas as pl
import jax.experimental.pallas.tpu as pltpu

_LANES = 128

_TP = 4
_S = 8
_D = 2048
_R = 16
_NA = 18
_LEAD = 2
_R0 = 64
_SPLIT = 4
_BURST = 32
_KW = 32


@jax.jit
def pallas_standalone__detection_seg_fpn_lateral__vision_kernel(
    c_fine: jax.Array,
    p_coarse: jax.Array,
    w_lat: jax.Array,
    w_out: jax.Array,
):
    B, H, W, C = c_fine.shape
    assert w_out.shape == (1, 1, C, C) and w_lat.shape == (C, C)
    assert p_coarse.shape == (B, H // 2, W // 2, C)
    dt = c_fine.dtype
    TP, S, D, R, NA, LEAD, R0 = _TP, _S, _D, _R, _NA, _LEAD, _R0
    M = B * H * W
    W2 = W // 2
    PR = 2 * W
    J = D // PR
    G = M // (S * D)
    SB = S // TP
    NU = G * J * SB
    PERS = PR // R
    NW = G * J * PERS
    NT = C // _LANES
    NPC = TP * PR // R0
    NPP = TP * W2 // R0
    assert G * S * D == M and J * PR == D and SB * TP == S and NT * _LANES == C
    assert W % _SPLIT == 0 and TP % _SPLIT == 0 and PR % R0 == 0 and W2 % R0 == 0
    assert NA + LEAD < NU - 1 and _KW % (2 * TP) == 0
    n_paced = _BURST + (NU - NA) * _KW
    assert _BURST <= (NA // SB) * PERS and n_paced <= ((NU - 1) // SB) * PERS

    SEM_W, SEM_REST, SEM_TAIL, SEM_C = 0, 2, 3, 4
    SEM_P = SEM_C + LEAD
    n_sem = SEM_P + LEAD

    def step_pos(u):
        slab = u // SB
        return slab // J, (u % SB) * TP, slab % J

    def boxes(a, b):
        out = []
        while a < b:
            g, s0, j = step_pos(a)
            if a % SB != 0 or b - a < SB:
                out.append((g, pl.ds(s0, TP), pl.ds(j, 1)))
                a += 1
            elif j == 0 and b - a >= SB * J:
                ng = (b - a) // (SB * J)
                out.append((pl.ds(g, ng),))
                a += ng * SB * J
            else:
                m = min(J - j, (b - a) // SB)
                out.append((g, slice(None), pl.ds(j, m)))
                a += m * SB
        return out

    def kernel(c_hbm, p_hbm, wl_hbm, wo_hbm, o_hbm,
               cbuf, pbuf, obuf, wl, wo, wf, qs, sem, osem):
        def c_copy(idx, s):
            return pltpu.make_async_copy(c_hbm.at[idx], cbuf.at[idx], sem.at[s])

        def p_copy(idx, s):
            return pltpu.make_async_copy(p_hbm.at[idx], pbuf.at[idx], sem.at[s])

        def step_copies(u):
            g, s0, j = step_pos(u)
            idx = (g, pl.ds(s0, TP), pl.ds(j, 1))
            return [p_copy(idx, SEM_P + u % LEAD), c_copy(idx, SEM_C + u % LEAD)]

        def out_copy(k):
            g = k // (J * PERS)
            off = pl.multiple_of((k % (J * PERS)) * R, R)
            return pltpu.make_async_copy(
                obuf.at[g, :, pl.ds(off, R)], o_hbm.at[g, :, pl.ds(off, R)], osem)

        w_copies = [pltpu.make_async_copy(wl_hbm, wl, sem.at[SEM_W]),
                    pltpu.make_async_copy(wo_hbm, wo, sem.at[SEM_W + 1])]
        rest = [p_copy(i, SEM_REST) for i in boxes(NA + LEAD, NU - 1)]
        rest += [c_copy(i, SEM_REST) for i in boxes(NA + LEAD, NU)]
        (tail,) = [p_copy(i, SEM_TAIL) for i in boxes(NU - 1, NU)]
        for d in w_copies:
            d.start(priority=0)
        for u in range(LEAD):
            for d in step_copies(u):
                d.start(priority=1)
        for d in rest + [tail]:
            d.start(priority=1)
        for d in w_copies:
            d.wait()
        wf[...] = jnp.dot(wl[...], wo[...],
                          preferred_element_type=jnp.float32).astype(dt)

        def store_q(n, qn):
            qs[n, pl.ds(0, TP * W2, stride=2), :] = qn
            qs[n, pl.ds(1, TP * W2, stride=2), :] = qn

        def split_dot(load, nrows, w_ref, anchor, emit):
            nb = nrows // _SPLIT
            for n in range(NT):
                parts = []
                for h in range(_SPLIT):
                    anchor(n * _SPLIT + h)
                    parts.append(load(h * nb, nb))
                emit(n, jnp.dot(jnp.concatenate(parts, axis=0),
                                w_ref[:, n * _LANES:(n + 1) * _LANES],
                                preferred_element_type=jnp.float32))

        def read_step(u, carry):
            for d in step_copies(u):
                d.wait()
            g, s0, j = step_pos(u)
            vg, vs0, vj = step_pos(u + LEAD)
            slot = u % LEAD
            na = NT * _SPLIT

            def p_anchor(a):
                per = W2 // R0
                for k in range(a * NPP // na, (a + 1) * NPP // na):
                    p_copy((vg, vs0 + k // per, vj, pl.ds((k % per) * R0, R0)),
                           SEM_P + slot).start(priority=0)

            def c_anchor(a):
                per = PR // R0
                tot = 2 * TP * na
                for k in range(a * NPC // tot, (a + 1) * NPC // tot):
                    c_copy((vg, vs0 + k // per, vj, pl.ds((k % per) * R0, R0)),
                           SEM_C + slot).start(priority=0)

            def load_p(r0, nr):
                return pbuf[g, pl.ds(s0 + r0 // W2, nr // W2), j].reshape(nr, C)

            split_dot(load_p, TP * W2, wo, p_anchor, store_q)
            for t in range(TP):
                for r in range(2):
                    rows = pl.ds(pl.multiple_of(j * PR + r * W, W), W)

                    def load_c(r0, nr):
                        return cbuf[g, s0 + t, j, pl.ds(r * W + r0, nr), :]

                    def emit(n, acc):
                        res = acc + qs[n, pl.ds(t * W, W), :]
                        obuf[g, s0 + t, rows, pl.ds(n * _LANES, _LANES)] = (
                            res.astype(dt))

                    split_dot(load_c, W, wf,
                              lambda a: c_anchor((2 * t + r) * na + a), emit)
            return carry

        lax.fori_loop(0, NA, read_step, 0)

        for u in range(NA, NA + LEAD):
            for d in step_copies(u):
                d.wait()
        for d in rest:
            d.wait()
        for k in range(_BURST):
            out_copy(k).start()
        tail.wait()

        def write_step(u, carry):
            g, s0, j = step_pos(u)
            base = _BURST + (u - NA) * _KW
            kh = _KW // (2 * TP)
            p = pbuf[g, pl.ds(s0, TP), j].reshape(TP * W2, C)
            q = jnp.dot(p, wo[...], preferred_element_type=jnp.float32)
            for n in range(NT):
                store_q(n, q[:, n * _LANES:(n + 1) * _LANES])
            for t in range(TP):
                for r in range(2):
                    rows = pl.ds(pl.multiple_of(j * PR + r * W, W), W)
                    c = cbuf[g, s0 + t, j, pl.ds(r * W, W), :]
                    up = jnp.concatenate(
                        [qs[n, pl.ds(t * W, W), :] for n in range(NT)], axis=1)
                    res = jnp.dot(c, wf[...],
                                  preferred_element_type=jnp.float32) + up
                    for k in range(kh):
                        out_copy(base + (2 * t + r) * kh + k).start()
                    obuf[g, s0 + t, rows, :] = res.astype(dt)
            return carry

        lax.fori_loop(NA, NU, write_step, 0)
        for k in range(n_paced, NW):
            out_copy(k).start()
        pltpu.make_async_copy(obuf, o_hbm, osem).wait()

    out = pl.pallas_call(
        kernel,
        in_specs=[pl.BlockSpec(memory_space=pl.ANY)] * 4,
        out_specs=pl.BlockSpec(memory_space=pl.ANY),
        out_shape=jax.ShapeDtypeStruct((G, S, D, C), dt),
        scratch_shapes=[
            pltpu.VMEM((G, S, J, PR, C), dt),
            pltpu.VMEM((G, S, J, W2, C), dt),
            pltpu.VMEM((G, S, D, C), dt),
            pltpu.VMEM((C, C), dt),
            pltpu.VMEM((C, C), dt),
            pltpu.VMEM((C, C), dt),
            pltpu.VMEM((NT, TP * W, _LANES), jnp.float32),
            pltpu.SemaphoreType.DMA((n_sem,)),
            pltpu.SemaphoreType.DMA,
        ],
        compiler_params=pltpu.CompilerParams(
            vmem_limit_bytes=124 * 1024 * 1024,
            disable_bounds_checks=True,
            disable_semaphore_checks=True,
        ),
    )(
        c_fine.reshape(G, S, J, PR, C),
        p_coarse.reshape(G, S, J, W2, C),
        w_lat,
        w_out.reshape(C, C),
    )
    return out.reshape(B, H, W, C)
```

```python
import jax
import jax.numpy as jnp
from jax import lax
import jax.experimental.pallas as pl
import jax.experimental.pallas.tpu as pltpu

_LANES = 128

_TP = 4
_S = 8
_D = 2048
_NA = 18
_LEAD = 2
_R_HI = 8
_R_LO = 64
_LO_PER_STEP = 4
_LO_START = 4
_P_CHUNKS = (2, 4, 12)
_SPLIT = 4
_R_OUT = 16
_BURST = 32
_KW = 32


def _div(x, n):
    if isinstance(x, int):
        return x // n
    assert n & (n - 1) == 0
    return lax.shift_right_logical(x, n.bit_length() - 1) if n > 1 else x


def _mod(x, n):
    if isinstance(x, int):
        return x % n
    assert n & (n - 1) == 0
    return lax.bitwise_and(x, n - 1)


@jax.jit
def pallas_standalone__detection_seg_fpn_lateral__vision_kernel(
    c_fine: jax.Array,
    p_coarse: jax.Array,
    w_lat: jax.Array,
    w_out: jax.Array,
):
    B, H, W, C = c_fine.shape
    assert w_out.shape == (1, 1, C, C) and w_lat.shape == (C, C)
    assert p_coarse.shape == (B, H // 2, W // 2, C)
    dt = c_fine.dtype
    TP, S, D, NA, LEAD = _TP, _S, _D, _NA, _LEAD
    M = B * H * W
    W2 = W // 2
    PR = 2 * W
    J = D // PR
    G = M // (S * D)
    SB = S // TP
    NU = G * J * SB
    NT = C // _LANES
    assert G * S * D == M and J * PR == D and SB * TP == S and NT * _LANES == C
    assert J == TP and J * W2 == PR and G * S == S * J and TP == _SPLIT

    n_hi = PR // _R_HI
    lo_slab0 = (NA + LEAD) // SB
    lo_per_slab = PR // _R_LO
    lo_steps = (G * J - lo_slab0) * lo_per_slab // _LO_PER_STEP
    assert (NA + LEAD) % SB == 0 and lo_per_slab % _LO_PER_STEP == 0
    assert _LO_START + lo_steps <= NA and _P_CHUNKS[0] == LEAD
    out_per_slab = PR // _R_OUT
    n_out = G * J * out_per_slab
    n_paced = _BURST + (NU - NA) * _KW
    assert _KW % (2 * TP) == 0 and _BURST <= (NA // SB) * out_per_slab
    assert n_paced <= ((NU - 1) // SB) * out_per_slab

    na = NT * _SPLIT
    cum = [0]
    for wgt in [2] * na + [1] * (2 * TP * na):
        cum.append(cum[-1] + wgt)

    def hi_pieces(a):
        return range(cum[a] * n_hi // cum[-1], cum[a + 1] * n_hi // cum[-1])

    SEM_W, SEM_LO, SEM_TAIL, SEM_C = 0, 2, 3, 4
    SEM_P = SEM_C + LEAD
    SEM_PC = SEM_P + LEAD
    n_sem = SEM_PC + len(_P_CHUNKS)

    def step_pos(u):
        slab = _div(u, SB)
        return _div(slab, J), _mod(u, SB) * TP, _mod(slab, J)

    def p_boxes(a, b):
        out = []
        while a < b:
            g, s0, j = step_pos(a)
            if a % SB != 0 or b - a < SB:
                out.append((pl.ds((g * S + s0) // J, 1), slice(None),
                            pl.ds(j * W2, W2)))
                a += 1
            elif j == 0 and b - a >= SB * J:
                ng = (b - a) // (SB * J)
                out.append((pl.ds(g * SB, ng * SB),))
                a += ng * SB * J
            else:
                m = min(J - j, (b - a) // SB)
                out.append((pl.ds(g * SB, SB), slice(None),
                            pl.ds(j * W2, m * W2)))
                a += m * SB
        return out

    def kernel(c_hbm, p_hbm, wl_hbm, wo_hbm, o_hbm,
               xbuf, obuf, wl, wo, wf, qs, sem, osem):
        def c_copy(idx, s):
            return pltpu.make_async_copy(c_hbm.at[idx], xbuf.at[idx], sem.at[s])

        def p_copy(idx, s):
            return pltpu.make_async_copy(
                p_hbm.at[idx], xbuf.at[(G,) + idx], sem.at[s])

        def c_step(u):
            g, s0, j = step_pos(u)
            return c_copy((g, pl.ds(s0, TP), j), SEM_C + _mod(u, LEAD))

        def p_step(u):
            g, s0, j = step_pos(u)
            rows = pl.ds(pl.multiple_of(j * W2, W2), W2)
            return p_copy((_div(g * S + s0, J), slice(None), rows), SEM_P + u)

        def out_copy(k):
            g = _div(k, J * out_per_slab)
            off = pl.multiple_of(_mod(k, J * out_per_slab) * _R_OUT, _R_OUT)
            rows = pl.ds(off, _R_OUT)
            return pltpu.make_async_copy(
                obuf.at[g, :, rows], o_hbm.at[g, :, rows], osem)

        w_copies = [pltpu.make_async_copy(wl_hbm, wl, sem.at[SEM_W]),
                    pltpu.make_async_copy(wo_hbm, wo, sem.at[SEM_W + 1])]
        bounds = list(_P_CHUNKS) + [NU - 1]
        p_chunks = [[p_copy(i, SEM_PC + k)
                     for i in p_boxes(bounds[k], bounds[k + 1])]
                    for k in range(len(_P_CHUNKS))]
        (tail,) = [p_copy(i, SEM_TAIL) for i in p_boxes(NU - 1, NU)]
        for d in w_copies:
            d.start(priority=0)
        for u in range(LEAD):
            p_step(u).start(priority=1)
            c_step(u).start(priority=1)
        for chunk in p_chunks:
            for d in chunk:
                d.start(priority=1)
        for d in w_copies:
            d.wait()
        wf[...] = jnp.dot(wl[...], wo[...],
                          preferred_element_type=jnp.float32).astype(dt)

        def store_q(n, qn):
            qs[n, pl.ds(0, TP * W2, stride=2), :] = qn
            qs[n, pl.ds(1, TP * W2, stride=2), :] = qn

        def split_dot(load, w_ref, anchor, emit):
            for n in range(NT):
                parts = []
                for h in range(_SPLIT):
                    anchor(n * _SPLIT + h)
                    parts.append(load(h))
                emit(n, jnp.dot(jnp.concatenate(parts, axis=0),
                                w_ref[:, n * _LANES:(n + 1) * _LANES],
                                preferred_element_type=jnp.float32))

        def read_step(u, carry):
            @pl.when(u < LEAD)
            def _():
                p_step(u).wait()

            for k, first in enumerate(_P_CHUNKS):
                @pl.when(u == first)
                def _(k=k):
                    for d in p_chunks[k]:
                        d.wait()

            @pl.when((u >= _LO_START) & (u < _LO_START + lo_steps))
            def _():
                it = u - _LO_START
                per = lo_per_slab // _LO_PER_STEP
                slab = lo_slab0 + _div(it, per)
                for i in range(_LO_PER_STEP):
                    off = (_mod(it, per) * _LO_PER_STEP + i) * _R_LO
                    rows = pl.ds(pl.multiple_of(off, _R_LO), _R_LO)
                    c_copy((_div(slab, J), slice(None), _mod(slab, J), rows),
                           SEM_LO).start(priority=1)

            c_step(u).wait()
            g, s0, j = step_pos(u)
            vg, vs0, vj = step_pos(u + LEAD)
            prow = pl.ds(pl.multiple_of(j * W2, W2), W2)
            nb = W // _SPLIT

            def anchor(a):
                for k in hi_pieces(a):
                    c_copy((vg, pl.ds(vs0, TP), vj, pl.ds(k * _R_HI, _R_HI)),
                           SEM_C + _mod(u, LEAD)).start(priority=0)

            split_dot(lambda h: xbuf[G, _div(g * S + s0, J), h, prow, :],
                      wo, anchor, store_q)
            for t in range(TP):
                for r in range(2):
                    rows = pl.ds(pl.multiple_of(j * PR + r * W, W), W)

                    def emit(n, acc):
                        res = acc + qs[n, pl.ds(t * W, W), :]
                        obuf[g, s0 + t, rows, pl.ds(n * _LANES, _LANES)] = (
                            res.astype(dt))

                    split_dot(
                        lambda h: xbuf[g, s0 + t, j, pl.ds(r * W + h * nb, nb), :],
                        wf, lambda a: anchor((1 + 2 * t + r) * na + a), emit)
            return carry

        lax.fori_loop(0, NA, read_step, 0)

        tail.start(priority=1)
        for u in range(NA, NA + LEAD):
            c_step(u).wait()
        for slab in range(lo_slab0, G * J):
            c_copy((slab // J, slice(None), slab % J), SEM_LO).wait()
        for k in range(_BURST):
            out_copy(k).start()
        tail.wait()

        def write_step(u, carry):
            g, s0, j = step_pos(u)
            base = _BURST + (u - NA) * _KW
            kh = _KW // (2 * TP)
            prow = pl.ds(pl.multiple_of(j * W2, W2), W2)
            p = xbuf[G, _div(g * S + s0, J), :, prow, :].reshape(TP * W2, C)
            q = jnp.dot(p, wo[...], preferred_element_type=jnp.float32)
            for n in range(NT):
                store_q(n, q[:, n * _LANES:(n + 1) * _LANES])
            for t in range(TP):
                for r in range(2):
                    rows = pl.ds(pl.multiple_of(j * PR + r * W, W), W)
                    c = xbuf[g, s0 + t, j, pl.ds(r * W, W), :]
                    up = jnp.concatenate(
                        [qs[n, pl.ds(t * W, W), :] for n in range(NT)], axis=1)
                    res = jnp.dot(c, wf[...],
                                  preferred_element_type=jnp.float32) + up
                    for k in range(kh):
                        out_copy(base + (2 * t + r) * kh + k).start()
                    obuf[g, s0 + t, rows, :] = res.astype(dt)
            return carry

        lax.fori_loop(NA, NU, write_step, 0)
        for k in range(n_paced, n_out):
            out_copy(k).start()
        pltpu.make_async_copy(obuf, o_hbm, osem).wait()

    out = pl.pallas_call(
        kernel,
        in_specs=[pl.BlockSpec(memory_space=pl.ANY)] * 4,
        out_specs=pl.BlockSpec(memory_space=pl.ANY),
        out_shape=jax.ShapeDtypeStruct((G, S, D, C), dt),
        scratch_shapes=[
            pltpu.VMEM((G + 1, S, J, PR, C), dt),
            pltpu.VMEM((G, S, D, C), dt),
            pltpu.VMEM((C, C), dt),
            pltpu.VMEM((C, C), dt),
            pltpu.VMEM((C, C), dt),
            pltpu.VMEM((NT, TP * W, _LANES), jnp.float32),
            pltpu.SemaphoreType.DMA((n_sem,)),
            pltpu.SemaphoreType.DMA,
        ],
        compiler_params=pltpu.CompilerParams(
            vmem_limit_bytes=124 * 1024 * 1024,
            disable_bounds_checks=True,
            disable_semaphore_checks=True,
        ),
    )(
        c_fine.reshape(G, S, J, PR, C),
        p_coarse.reshape(S, J, PR, C),
        w_lat,
        w_out.reshape(C, C),
    )
    return out.reshape(B, H, W, C)
```

```python
import jax
import jax.numpy as jnp
from jax import lax
import jax.experimental.pallas as pl
import jax.experimental.pallas.tpu as pltpu

_LANES = 128

_TP = 4
_S = 8
_D = 2048
_NA = 18
_LEAD = 2
_R_HI = 16
_R_LO = 64
_LO_PER_STEP = 4
_LO_START = 4
_P_CHUNKS = (2, 4, 12)
_SPLIT = 4
_R_OUT = 16
_BURST = 32
_KW = 32


def _div(x, n):
    if isinstance(x, int):
        return x // n
    assert n & (n - 1) == 0
    return lax.shift_right_logical(x, n.bit_length() - 1) if n > 1 else x


def _mod(x, n):
    if isinstance(x, int):
        return x % n
    assert n & (n - 1) == 0
    return lax.bitwise_and(x, n - 1)


@jax.jit
def pallas_standalone__detection_seg_fpn_lateral__vision_kernel(
    c_fine: jax.Array,
    p_coarse: jax.Array,
    w_lat: jax.Array,
    w_out: jax.Array,
):
    B, H, W, C = c_fine.shape
    assert w_out.shape == (1, 1, C, C) and w_lat.shape == (C, C)
    assert p_coarse.shape == (B, H // 2, W // 2, C)
    dt = c_fine.dtype
    TP, S, D, NA, LEAD = _TP, _S, _D, _NA, _LEAD
    M = B * H * W
    W2 = W // 2
    PR = 2 * W
    J = D // PR
    G = M // (S * D)
    SB = S // TP
    NU = G * J * SB
    NT = C // _LANES
    assert G * S * D == M and J * PR == D and SB * TP == S and NT * _LANES == C
    assert J == TP and J * W2 == PR and G * S == S * J and TP == _SPLIT

    n_hi = PR // _R_HI
    lo_slab0 = (NA + LEAD) // SB
    lo_per_slab = PR // _R_LO
    lo_steps = (G * J - lo_slab0) * lo_per_slab // _LO_PER_STEP
    assert (NA + LEAD) % SB == 0 and lo_per_slab % _LO_PER_STEP == 0
    assert _LO_START + lo_steps <= NA and _P_CHUNKS[0] == LEAD
    out_per_slab = PR // _R_OUT
    n_out = G * J * out_per_slab
    n_paced = _BURST + (NU - NA) * _KW
    assert _KW % (2 * TP) == 0 and _BURST <= (NA // SB) * out_per_slab
    assert n_paced <= ((NU - 1) // SB) * out_per_slab

    na = NT * _SPLIT
    cum = [0]
    for wgt in [2] * na + [1] * (2 * TP * na):
        cum.append(cum[-1] + wgt)

    def hi_pieces(a):
        return range(cum[a] * n_hi // cum[-1], cum[a + 1] * n_hi // cum[-1])

    SEM_W, SEM_LO, SEM_TAIL, SEM_C = 0, 2, 3, 4
    SEM_P = SEM_C + LEAD
    SEM_PC = SEM_P + LEAD
    n_sem = SEM_PC + len(_P_CHUNKS)

    def step_pos(u):
        slab = _div(u, SB)
        return _div(slab, J), _mod(u, SB) * TP, _mod(slab, J)

    def p_boxes(a, b):
        out = []
        while a < b:
            g, s0, j = step_pos(a)
            if a % SB != 0 or b - a < SB:
                out.append((pl.ds((g * S + s0) // J, 1), slice(None),
                            pl.ds(j * W2, W2)))
                a += 1
            elif j == 0 and b - a >= SB * J:
                ng = (b - a) // (SB * J)
                out.append((pl.ds(g * SB, ng * SB),))
                a += ng * SB * J
            else:
                m = min(J - j, (b - a) // SB)
                out.append((pl.ds(g * SB, SB), slice(None),
                            pl.ds(j * W2, m * W2)))
                a += m * SB
        return out

    def kernel(c_hbm, p_hbm, wl_hbm, wo_hbm, o_hbm,
               xbuf, obuf, wl, wo, wf, qs, sem, osem):
        def c_copy(idx, s):
            return pltpu.make_async_copy(c_hbm.at[idx], xbuf.at[idx], sem.at[s])

        def p_copy(idx, s):
            return pltpu.make_async_copy(
                p_hbm.at[idx], xbuf.at[(G,) + idx], sem.at[s])

        def c_step(u):
            g, s0, j = step_pos(u)
            return c_copy((g, pl.ds(s0, TP), j), SEM_C + _mod(u, LEAD))

        def p_step(u):
            g, s0, j = step_pos(u)
            rows = pl.ds(pl.multiple_of(j * W2, W2), W2)
            return p_copy((_div(g * S + s0, J), slice(None), rows), SEM_P + u)

        def lo_copy(it, i):
            per = lo_per_slab // _LO_PER_STEP
            slab = lo_slab0 + _div(it, per)
            off = (_mod(it, per) * _LO_PER_STEP + i) * _R_LO
            rows = pl.ds(pl.multiple_of(off, _R_LO), _R_LO)
            return c_copy((_div(slab, J), slice(None), _mod(slab, J), rows),
                          SEM_LO)

        def out_copy(k):
            g = _div(k, J * out_per_slab)
            off = pl.multiple_of(_mod(k, J * out_per_slab) * _R_OUT, _R_OUT)
            rows = pl.ds(off, _R_OUT)
            return pltpu.make_async_copy(
                obuf.at[g, :, rows], o_hbm.at[g, :, rows], osem)

        w_copies = [pltpu.make_async_copy(wl_hbm, wl, sem.at[SEM_W]),
                    pltpu.make_async_copy(wo_hbm, wo, sem.at[SEM_W + 1])]
        bounds = list(_P_CHUNKS) + [NU - 1]
        p_chunks = [[p_copy(i, SEM_PC + k)
                     for i in p_boxes(bounds[k], bounds[k + 1])]
                    for k in range(len(_P_CHUNKS))]
        (tail,) = [p_copy(i, SEM_TAIL) for i in p_boxes(NU - 1, NU)]
        for d in w_copies:
            d.start(priority=0)
        for u in range(LEAD):
            p_step(u).start(priority=1)
            c_step(u).start(priority=1)
        for chunk in p_chunks:
            for d in chunk:
                d.start(priority=1)
        qs[...] = jnp.zeros(qs.shape, qs.dtype)
        for d in w_copies:
            d.wait()
        wf[...] = jnp.dot(wl[...], wo[...],
                          preferred_element_type=jnp.float32).astype(dt)

        def store_q(n, qn):
            qs[n, pl.ds(0, TP * W2, stride=2), :] = qn
            qs[n, pl.ds(1, TP * W2, stride=2), :] = qn

        def split_dot(load, w_ref, anchor, emit):
            for n in range(NT):
                parts = []
                for h in range(_SPLIT):
                    anchor(n * _SPLIT + h)
                    parts.append(load(h))
                emit(n, jnp.dot(jnp.concatenate(parts, axis=0),
                                w_ref[:, n * _LANES:(n + 1) * _LANES],
                                preferred_element_type=jnp.float32))

        def read_step(u, carry):
            @pl.when(u < LEAD)
            def _():
                p_step(u).wait()

            for k, first in enumerate(_P_CHUNKS):
                @pl.when(u == first)
                def _(k=k):
                    for d in p_chunks[k]:
                        d.wait()

            @pl.when((u >= _LO_START) & (u < _LO_START + lo_steps))
            def _():
                for i in range(_LO_PER_STEP):
                    lo_copy(u - _LO_START, i).start(priority=1)

            c_step(u).wait()
            g, s0, j = step_pos(u)
            vg, vs0, vj = step_pos(u + LEAD)
            prow = pl.ds(pl.multiple_of(j * W2, W2), W2)
            nb = W // _SPLIT

            def anchor(a):
                for k in hi_pieces(a):
                    c_copy((vg, pl.ds(vs0, TP), vj, pl.ds(k * _R_HI, _R_HI)),
                           SEM_C + _mod(u, LEAD)).start(priority=0)

            split_dot(lambda h: xbuf[G, _div(g * S + s0, J), h, prow, :],
                      wo, anchor, store_q)
            for t in range(TP):
                for r in range(2):
                    rows = pl.ds(pl.multiple_of(j * PR + r * W, W), W)

                    def emit(n, acc):
                        res = acc + qs[n, pl.ds(t * W, W), :]
                        obuf[g, s0 + t, rows, pl.ds(n * _LANES, _LANES)] = (
                            res.astype(dt))

                    split_dot(
                        lambda h: xbuf[g, s0 + t, j, pl.ds(r * W + h * nb, nb), :],
                        wf, lambda a: anchor((1 + 2 * t + r) * na + a), emit)
            return carry

        lax.fori_loop(0, NA, read_step, 0)

        tail.start(priority=1)
        for u in range(NA, NA + LEAD):
            c_step(u).wait()
        for it in range(lo_steps):
            for i in range(_LO_PER_STEP):
                lo_copy(it, i).wait()
        for k in range(_BURST):
            out_copy(k).start()
        tail.wait()

        def write_step(u, carry):
            g, s0, j = step_pos(u)
            base = _BURST + (u - NA) * _KW
            kh = _KW // (2 * TP)
            prow = pl.ds(pl.multiple_of(j * W2, W2), W2)
            p = xbuf[G, _div(g * S + s0, J), :, prow, :].reshape(TP * W2, C)
            q = jnp.dot(p, wo[...], preferred_element_type=jnp.float32)
            for n in range(NT):
                store_q(n, q[:, n * _LANES:(n + 1) * _LANES])
            for t in range(TP):
                for r in range(2):
                    rows = pl.ds(pl.multiple_of(j * PR + r * W, W), W)
                    c = xbuf[g, s0 + t, j, pl.ds(r * W, W), :]
                    up = jnp.concatenate(
                        [qs[n, pl.ds(t * W, W), :] for n in range(NT)], axis=1)
                    res = jnp.dot(c, wf[...],
                                  preferred_element_type=jnp.float32) + up
                    for k in range(kh):
                        out_copy(base + (2 * t + r) * kh + k).start()
                    obuf[g, s0 + t, rows, :] = res.astype(dt)
            return carry

        lax.fori_loop(NA, NU, write_step, 0)
        for k in range(n_paced, n_out):
            out_copy(k).start()
        pltpu.make_async_copy(obuf, o_hbm, osem).wait()

    out = pl.pallas_call(
        kernel,
        in_specs=[pl.BlockSpec(memory_space=pl.ANY)] * 4,
        out_specs=pl.BlockSpec(memory_space=pl.ANY),
        out_shape=jax.ShapeDtypeStruct((G, S, D, C), dt),
        scratch_shapes=[
            pltpu.VMEM((G + 1, S, J, PR, C), dt),
            pltpu.VMEM((G, S, D, C), dt),
            pltpu.VMEM((C, C), dt),
            pltpu.VMEM((C, C), dt),
            pltpu.VMEM((C, C), dt),
            pltpu.VMEM((NT, TP * W + 8, _LANES), jnp.float32),
            pltpu.SemaphoreType.DMA((n_sem,)),
            pltpu.SemaphoreType.DMA,
        ],
        compiler_params=pltpu.CompilerParams(
            vmem_limit_bytes=124 * 1024 * 1024,
            disable_bounds_checks=True,
            disable_semaphore_checks=True,
        ),
    )(
        c_fine.reshape(G, S, J, PR, C),
        p_coarse.reshape(S, J, PR, C),
        w_lat,
        w_out.reshape(C, C),
    )
    return out.reshape(B, H, W, C)
```
